```python
import os as _os
_os.environ.setdefault("JAX_PLATFORMS", "cpu")
import jax
import jax.numpy as jnp

def _softmax(x, axis=-1):
    return jax.nn.softmax(x, axis=axis)
def _gelu(x):
    return jax.nn.gelu(x, approximate=True)
def _silu(x):
    return jax.nn.silu(x)
def _sigmoid(x):
    return jax.nn.sigmoid(x)
def _layernorm(x, axis=-1, eps=1e-5):
    m = jnp.mean(x, axis=axis, keepdims=True)
    v = jnp.var(x, axis=axis, keepdims=True)
    return (x - m) / jnp.sqrt(v + eps)
def _scatter_add(tgt, idx, src, axis=0):
    return tgt.at[idx].add(src)
def _segment_sum(src, seg, n):
    return jax.ops.segment_sum(src, seg, n)
class _Rng:
    def __init__(self, key):
        self._k = key
    def _next(self):
        self._k, sub = jax.random.split(self._k)
        return sub
    def normal(self, shape):
        return jax.random.normal(self._next(), shape, dtype=jnp.bfloat16)
    def randint(self, lo, hi, shape):
        return jax.random.randint(self._next(), shape, lo, hi, dtype=jnp.int32)
    def uniform(self, shape, lo=0.0, hi=1.0):
        return jax.random.uniform(self._next(), shape, jnp.bfloat16, lo, hi)
    def permutation(self, n):
        return jax.random.permutation(self._next(), n)


kernel_name = 'parallel_sum__linear_kernel_hedgehog__dense_activation_gelu__prompt'

def setup_inputs():
    _rng = _Rng(jax.random.key(int.from_bytes(__import__("os").urandom(4), "little")))
    _w = (lambda a: (lambda t: t.astype(jnp.bfloat16) if jnp.issubdtype(t.dtype, jnp.floating) else t)(jnp.asarray(a)))
    def _A_setup():
        B, S, D, H = 1, 2048, 448, 16
        Dh = D // H
        return {
            "x": _w((lambda *s: _rng.normal(s) * 0.05)(B, S, D)),
            "wqkv": _w((lambda *s: _rng.normal(s) * 0.2)(D, 3 * D)),
            "w_phi": _w((lambda *s: _rng.normal(s) * 0.2)(H, Dh, Dh) * (Dh ** -0.5)),
            "wo": _w((lambda *s: _rng.normal(s) * 0.05)(D, D)),
        }
    _A_in = _A_setup()

    def _B_setup():
        B, S, D, F = 1, 2048, 448, 1792
        return {
            "x": _w((lambda *s: _rng.normal(s) * 0.05)(B, S, D)),
            "w1": _w((lambda *s: _rng.normal(s) * 0.2)(D, F) * (D ** -0.5)),
            "b1": _w((lambda *s: _rng.normal(s) * 0.2)(F) * 0.01),
            "w2": _w((lambda *s: _rng.normal(s) * 0.2)(F, D) * (F ** -0.5)),
            "b2": _w((lambda *s: _rng.normal(s) * 0.05)(D) * 0.01),
        }
    _B_in = _B_setup()

    return {
        "A_x": _A_in["x"],
        "A_wqkv": _A_in["wqkv"],
        "A_w_phi": _A_in["w_phi"],
        "A_wo": _A_in["wo"],
        "B_x": _B_in["x"],
        "B_w1": _B_in["w1"],
        "B_b1": _B_in["b1"],
        "B_w2": _B_in["w2"],
        "B_b2": _B_in["b2"],
    }

def reference(A_x, A_wqkv, A_w_phi, A_wo, B_x, B_w1, B_b1, B_w2, B_b2):
    def _A_ref(x, wqkv, w_phi, wo):
        B, S, D = x.shape
        H = 16; Dh = D // H
        qkv = (lambda x, *d: x.transpose(*d))((x @ wqkv).reshape(B, S, 3, H, Dh), 2, 0, 3, 1, 4)
        q, k, v = qkv[0], qkv[1], qkv[2]
        pq = jnp.einsum("bhsd,hdf->bhsf", q, w_phi)
        pk = jnp.einsum("bhsd,hdf->bhsf", k, w_phi)
        phi_q = jnp.concatenate([_softmax(pq, axis=-1), _softmax(-pq, axis=-1)], axis=-1)
        phi_k = jnp.concatenate([_softmax(pk, axis=-1), _softmax(-pk, axis=-1)], axis=-1)
        kv = jnp.einsum("bhsf,bhsd->bhfd", phi_k, v)
        z  = jnp.einsum("bhsf->bhf", phi_k)
        num = jnp.einsum("bhqf,bhfd->bhqd", phi_q, kv)
        den = jnp.einsum("bhqf,bhf->bhq", phi_q, z)[..., None] + 1e-6
        o = num / den
        return (lambda x, *d: x.transpose(*d))(o, 0, 2, 1, 3).reshape(B, S, D) @ wo

    def _B_ref(x, w1, b1, w2, b2):
        h = jnp.einsum("bsd,df->bsf", x, w1) + b1
        h = _gelu(h)
        return jnp.einsum("bsf,fd->bsd", h, w2) + b2

    x = A_x
    xn = _layernorm(x, axis=-1)
    return x + _A_ref(xn, A_wqkv, A_w_phi, A_wo) + _B_ref(xn, B_w1, B_b1, B_w2, B_b2)
```

```python
import numpy as np
import jax
import jax.numpy as jnp
from jax import lax
import jax.experimental.pallas as pl
import jax.experimental.pallas.tpu as pltpu

S, D, H, DH, F = 2048, 448, 16, 28, 1792
G, GR = 4, 112
KX = 464
TT = 512
NT = S // TT
K2 = F + G * 128
BF, F32 = jnp.bfloat16, jnp.float32
NTD = (((1,), (1,)), ((), ()))
LCH = 512
LOG2E = 1.4426950408889634
KCH = 768
FCH = 256


def _dot(a, b):
    return jnp.dot(a, b, preferred_element_type=F32)


def _iota(shape, d):
    return lax.broadcasted_iota(jnp.int32, shape, d)


def _phi(p):
    n = p.shape[1]
    p3 = p.reshape(14, 8, n)
    mx = jnp.max(p3, axis=0)
    mn = jnp.min(p3, axis=0)
    mx = jnp.maximum(mx, pltpu.roll(mx, 4, 0))
    mn = jnp.minimum(mn, pltpu.roll(mn, 4, 0))
    ep = jnp.exp2(p3 - mx[None])
    en = jnp.exp2(mn[None] - p3)
    sp = jnp.sum(ep, axis=0)
    sn = jnp.sum(en, axis=0)
    sp = sp + pltpu.roll(sp, 4, 0)
    sn = sn + pltpu.roll(sn, 4, 0)
    a = (ep * (1.0 / sp)[None]).reshape(GR, n)
    b = (en * (1.0 / sn)[None]).reshape(GR, n)
    return a, b


def _gelu(x):
    c = 0.7978845608028654
    u = x * (c + (c * 0.044715) * (x * x))
    hx = 0.5 * x
    return hx + hx * jnp.tanh(u)


def _kernel(x_hbm, wqkv_hbm, wphi_ref, wo_hbm, w1_hbm, b1_ref, w2_hbm, b2_ref, o_hbm,
            x_v, wqkv_v, wqkvT, wo_v, w1_v, w2_v, lhs1, lhs2, lhs3, xnT,
            p_v, v_v, phi_v, p_w, v_w, phi_w, kv_acc, kvT, acts, out_v, sems, osems):
    cp = pltpu.make_async_copy
    QS = 384
    c_wqkv = cp(wqkv_hbm.at[:, pl.ds(QS, 3 * D - QS)], wqkv_v.at[pl.ds(0, D), pl.ds(QS, 3 * D - QS)], sems.at[0])
    c_wq = cp(wqkv_hbm.at[:, pl.ds(0, QS)], wqkv_v.at[pl.ds(0, D), pl.ds(0, QS)], sems.at[4 + NT])
    c_x = [cp(x_hbm.at[:, pl.ds(t * TT, TT)], x_v.at[t], sems.at[1 + t]) for t in range(NT)]
    c_w1 = cp(w1_hbm, w1_v.at[pl.ds(0, D)], sems.at[1 + NT])
    c_w2 = cp(w2_hbm, w2_v, sems.at[2 + NT])
    c_wo = cp(wo_hbm, wo_v, sems.at[3 + NT])
    c_wqkv.start()
    c_x[0].start()

    wqkv_v[pl.ds(D, 16), :] = jnp.zeros((16, 3 * D), BF)
    b1 = b1_ref[...].astype(F32).reshape(1, F)
    w1_v[pl.ds(D, 16), :] = jnp.where(_iota((16, F), 0) == 0, b1, 0.0).astype(BF)
    one16 = jnp.where(_iota((16, TT), 0) == 0, 1.0, 0.0).astype(BF)
    for g in range(G):
        acts[pl.ds(F + 128 * g + GR, 16), :] = one16
        for vb in (v_v, v_w):
            vb[g, pl.ds(GR, 16), :] = jnp.where(_iota((16, TT), 0) < 8, 1.0, 0.0).astype(BF)
    kv_acc[...] = jnp.zeros(kv_acc.shape, F32)

    r = _iota((GR, GR), 0)
    k = _iota((GR, GR), 1)
    hr = r & 3
    same = (k >= DH * hr) & (k < DH * hr + DH)
    perm = jnp.where(k == DH * hr + (r >> 2), 1.0, 0.0).astype(BF)
    expand = jnp.where(_iota((GR, DH), 1) == (_iota((GR, DH), 0) >> 2), 1.0, 0.0).astype(BF)
    bmat = []
    for g in range(G):
        kk = _iota((GR, D), 0)
        hh = (kk >= DH).astype(jnp.int32) + (kk >= 2 * DH).astype(jnp.int32) + (kk >= 3 * DH).astype(jnp.int32)
        sel = jnp.where(_iota((GR, D), 1) == (kk - DH * hh) * H + 4 * g + hh, 1.0, 0.0).astype(BF)
        wst = _dot(sel, wphi_ref[...]).astype(BF)
        b = lax.dot_general(expand, wst, NTD, preferred_element_type=F32)
        bmat.append(jnp.where(same, b, 0.0).astype(BF))

    def norm(t):
        for c in range(TT // LCH):
            ln = pl.ds(c * LCH, LCH)
            xt = x_v[t, :, ln].astype(F32)
            m = jnp.mean(xt, axis=0, keepdims=True)
            xc = xt - m
            var = jnp.mean(xc * xc, axis=0, keepdims=True)
            xnT[t, pl.ds(0, D), ln] = (xc * lax.rsqrt(var + 1e-5)).astype(BF)
        xnT[t, pl.ds(D, 16), :] = one16

    c_x[0].wait()
    norm(0)
    c_wqkv.wait()
    for c in c_x[1:]:
        c.start()
    c_wq.start()
    c_w1.start()
    c_wo.start()
    c_w2.start()
    wqkvT[pl.ds(QS, 3 * D - QS), :] = wqkv_v[:, pl.ds(QS, 3 * D - QS)].T
    for g in range(G):
        lhs1[pl.ds(GR * g, GR), :] = (LOG2E * _dot(bmat[g], wqkvT[pl.ds(D + GR * g, GR), :])).astype(BF)
    for g in range(G):
        lhs1[pl.ds(D + GR * g, GR), :] = _dot(perm, wqkvT[pl.ds(2 * D + GR * g, GR), :]).astype(BF)

    def feats(g, p_v=p_v, phi_v=phi_v):
        for c in range(TT // LCH):
            a, b = _phi(p_v[pl.ds(GR * g, GR), pl.ds(c * LCH, LCH)])
            phi_v[g, pl.ds(0, GR), pl.ds(c * LCH, LCH)] = a.astype(BF)
            phi_v[g, pl.ds(GR, GR), pl.ds(c * LCH, LCH)] = b.astype(BF)

    def kvdot(t):
        vb, fb = (v_v, phi_v) if t % 2 == 0 else (v_w, phi_w)
        for g in range(G):
            kv_acc[g] += lax.dot_general(fb[g], vb[g], NTD, preferred_element_type=F32)

    for t in range(NT):
        xn = xnT[t]
        pb, vb, fb = (p_v, v_v, phi_v) if t % 2 == 0 else (p_w, v_w, phi_w)
        pb[...] = _dot(lhs1[pl.ds(0, D), :], xn)
        if t == 0:
            for c in c_x[1:]:
                c.wait()
        if t == 2:
            c_wq.wait()
            c_w1.wait()
            c_w2.wait()
            c_wo.wait()
        if t + 1 < NT:
            norm(t + 1)
        if t > 0:
            kvdot(t - 1)
        for g in range(G):
            vb[g, pl.ds(0, GR), :] = _dot(lhs1[pl.ds(D + GR * g, GR), :], xn).astype(BF)
            feats(g, pb, fb)
        if t == 2:
            wqkvT[pl.ds(0, QS), :] = wqkv_v[:, pl.ds(0, QS)].T
            for g in range(G):
                lhs2[pl.ds(GR * g, GR), :] = (LOG2E * _dot(bmat[g], wqkvT[pl.ds(GR * g, GR), :])).astype(BF)
            lhs2[pl.ds(D, F), :] = w1_v[...].T
        if t == 3:
            for c in range(F // 256):
                lhs3[:, pl.ds(c * 256, 256)] = w2_v[:, pl.ds(c * 256, 256)]
            for g in range(G):
                wp = _dot(perm, wo_v[pl.ds(GR * g, GR), :])
                tail = jnp.zeros((16, D), F32)
                if g == 0:
                    tail = jnp.where(_iota((16, D), 0) == 0, b2_ref[...].astype(F32).reshape(1, D), 0.0)
                lhs3[:, pl.ds(F + 128 * g, 128)] = jnp.concatenate([wp, tail], axis=0).T.astype(BF)
    kvdot(NT - 1)

    hmask = (_iota((2 * GR, 128), 0) & 3) == (_iota((2 * GR, 128), 1) & 3)
    for g in range(G):
        kvT[g] = jnp.where(hmask, kv_acc[g], 0.0).T.astype(BF)

    def out_copy(t, slot):
        return cp(out_v.at[slot], o_hbm.at[:, pl.ds(pl.multiple_of(t * TT, TT), TT)], osems.at[slot])

    def tile(t, carry):
        slot = t % 2
        xn = xnT[t]
        p_v[...] = _dot(lhs2[pl.ds(0, D), :], xn)
        nch = F // FCH

        def ffn(i):
            h = _dot(lhs2[pl.ds(D + i * FCH, FCH), :], xn)
            acts[pl.ds(i * FCH, FCH), :] = _gelu(h).astype(BF)

        for g in range(G):
            ffn(g)
            feats(g)
        for g in range(G):
            nd = _dot(kvT[g], phi_v[g])
            rden = 1.0 / (nd[GR:GR + 8] + 1e-6)
            o = nd[:GR].reshape(14, 8, TT) * rden[None]
            acts[pl.ds(F + 128 * g, GR), :] = o.reshape(GR, TT).astype(BF)
        for i in range(G, nch):
            ffn(i)
        yt = None
        for c in range(K2 // KCH):
            d = _dot(lhs3[:, pl.ds(c * KCH, KCH)], acts[pl.ds(c * KCH, KCH), :])
            yt = d if yt is None else yt + d

        @pl.when(t >= 2)
        def _():
            out_copy(t - 2, slot).wait()

        out_v[slot] = (yt + x_v[t].astype(F32)).astype(BF)
        out_copy(t, slot).start()
        return carry

    lax.fori_loop(0, NT, tile, 0)
    for t in range(NT - 2, NT):
        out_copy(t, t % 2).wait()


@jax.jit
def pallas_parallel_sum__linear_kernel_hedgehog__dense_activation_gelu__prompt_kernel(
        A_x, A_wqkv, A_w_phi, A_wo, B_x, B_w1, B_b1, B_w2, B_b2):
    hbm = pl.BlockSpec(memory_space=pltpu.MemorySpace.HBM)
    vm = pl.BlockSpec(memory_space=pltpu.VMEM)
    out = pl.pallas_call(
        _kernel,
        out_shape=jax.ShapeDtypeStruct((D, S), BF),
        in_specs=[hbm, hbm, vm, hbm, hbm, vm, hbm, vm],
        out_specs=hbm,
        scratch_shapes=[
            pltpu.VMEM((NT, D, TT), BF),
            pltpu.VMEM((KX, 3 * D), BF),
            pltpu.VMEM((3 * D, KX), BF),
            pltpu.VMEM((D, D), BF),
            pltpu.VMEM((KX, F), BF),
            pltpu.VMEM((D, F), BF),
            pltpu.VMEM((2 * D, KX), BF),
            pltpu.VMEM((D + F, KX), BF),
            pltpu.VMEM((D, K2), BF),
            pltpu.VMEM((NT, KX, TT), BF),
            pltpu.VMEM((D, TT), F32),
            pltpu.VMEM((G, 128, TT), BF),
            pltpu.VMEM((G, 2 * GR, TT), BF),
            pltpu.VMEM((D, TT), F32),
            pltpu.VMEM((G, 128, TT), BF),
            pltpu.VMEM((G, 2 * GR, TT), BF),
            pltpu.VMEM((G, 2 * GR, 128), F32),
            pltpu.VMEM((G, 128, 2 * GR), BF),
            pltpu.VMEM((K2, TT), BF),
            pltpu.VMEM((2, D, TT), BF),
            pltpu.SemaphoreType.DMA((5 + NT,)),
            pltpu.SemaphoreType.DMA((2,)),
        ],
        compiler_params=pltpu.CompilerParams(vmem_limit_bytes=100 * 1024 * 1024),
    )(A_x.reshape(S, D).T, A_wqkv, A_w_phi.transpose(1, 0, 2).reshape(D, DH), A_wo, B_w1, B_b1, B_w2.T, B_b2)
    return out.T.reshape(1, S, D)
```
